```python
import jax
import jax.numpy as jnp

def _softmax(x, axis=-1):
    return jax.nn.softmax(x, axis=axis)
def _gelu(x):
    return jax.nn.gelu(x, approximate=True)
def _silu(x):
    return jax.nn.silu(x)
def _sigmoid(x):
    return jax.nn.sigmoid(x)
def _layernorm(x, axis=-1, eps=1e-5):
    m = jnp.mean(x, axis=axis, keepdims=True)
    v = jnp.var(x, axis=axis, keepdims=True)
    return (x - m) / jnp.sqrt(v + eps)
def _scatter_add(tgt, idx, src, axis=0):
    return tgt.at[idx].add(src)
def _segment_sum(src, seg, n):
    return jax.ops.segment_sum(src, seg, n)
class _Rng:
    def __init__(self, key):
        self._k = key
    def _next(self):
        self._k, sub = jax.random.split(self._k)
        return sub
    def normal(self, shape):
        return jax.random.normal(self._next(), shape, dtype=jnp.bfloat16)
    def randint(self, lo, hi, shape):
        return jax.random.randint(self._next(), shape, lo, hi, dtype=jnp.int32)
    def uniform(self, shape, lo=0.0, hi=1.0):
        return jax.random.uniform(self._next(), shape, jnp.bfloat16, lo, hi)
    def permutation(self, n):
        return jax.random.permutation(self._next(), n)


kernel_name = 'sequential_preLN__sliding_block__glu_gated_glu__prompt'

def _fwd_setup_inputs():
    _rng = _Rng(jax.random.key(int.from_bytes(__import__("os").urandom(4), "little")))
    _w = (lambda a: (lambda t: t.astype(jnp.bfloat16) if jnp.issubdtype(t.dtype, jnp.floating) else t)(jnp.asarray(a)))
    def _A_setup():
        B, S, D = 1, 2048, 512
        return {
            "x": _w((lambda *s: _rng.normal(s) * 0.05)(B, S, D)),
            "wqkv": _w((lambda *s: _rng.normal(s) * 0.05)(D, 3 * D)),
            "wo": _w((lambda *s: _rng.normal(s) * 0.05)(D, D)),
        }
    _A_in = _A_setup()

    def _B_setup():
        B, S, D, F = 1, 2048, 512, 1376
        return {
            "x": _w((lambda *s: _rng.normal(s) * 0.05)(B, S, D)),
            "w_gate": _w((lambda *s: _rng.normal(s) * 0.05)(D, F)),
            "w_up": _w((lambda *s: _rng.normal(s) * 0.05)(D, F)),
            "w_down": _w((lambda *s: _rng.normal(s) * 0.05)(F, D)),
        }
    _B_in = _B_setup()

    return {
        "A_x": _A_in["x"],
        "A_wqkv": _A_in["wqkv"],
        "A_wo": _A_in["wo"],
        "B_x": _B_in["x"],
        "B_w_gate": _B_in["w_gate"],
        "B_w_up": _B_in["w_up"],
        "B_w_down": _B_in["w_down"],
    }

def _fwd_reference(A_x, A_wqkv, A_wo, B_x, B_w_gate, B_w_up, B_w_down):
    def _A_ref(x, wqkv, wo):
        B, S, D = x.shape
        H = 32; Dh = D // H; W = 256
        qkv = (lambda x, *d: x.transpose(*d))((x @ wqkv).reshape(B, S, 3, H, Dh), 2, 0, 3, 1, 4)
        q, k, v = qkv[0], qkv[1], qkv[2]
        scores = jnp.einsum("bhqd,bhkd->bhqk", q, k) * (Dh ** -0.5)
        idx = jnp.arange(S)
        mask = (idx[:, None] - idx[None, :] >= 0) & (idx[:, None] - idx[None, :] < W)
        scores = jnp.where(mask[None, None], scores, -1e9)
        p = _softmax(scores, axis=-1)
        o = jnp.einsum("bhqk,bhkd->bhqd", p, v)
        return (lambda x, *d: x.transpose(*d))(o, 0, 2, 1, 3).reshape(B, S, D) @ wo

    def _B_ref(x, w_gate, w_up, w_down):
        g = jnp.einsum("bsd,df->bsf", x, w_gate)
        u = jnp.einsum("bsd,df->bsf", x, w_up)
        h = _sigmoid(g) * u
        return jnp.einsum("bsf,fd->bsd", h, w_down)

    x = A_x
    h = x + _A_ref(_layernorm(x, axis=-1), A_wqkv, A_wo)
    h2 = h + _B_ref(_layernorm(h, axis=-1), B_w_gate, B_w_up, B_w_down)
    return h2


def setup_inputs():
    _inp = _fwd_setup_inputs()
    _gk = jax.random.fold_in(jax.random.key(int.from_bytes(__import__("os").urandom(4), "little")), 2**31 - 1)
    _shapes = [[1, 2048, 512]]
    _dtypes = ['bfloat16']
    _gks = jax.random.split(_gk, len(_shapes))
    _gs = [jax.random.normal(k, s, dtype=jnp.dtype(d)) * 0.05 for k, s, d in zip(_gks, _shapes, _dtypes)]
    _inp["grad_out"] = _gs[0]
    return _inp

def reference(A_x, A_wqkv, A_wo, B_w_gate, B_w_up, B_w_down, B_x, grad_out):
    _const = dict(B_x=B_x)
    def _f(*_d):
        return _fwd_reference(**{'A_x': _d[0], 'A_wqkv': _d[1], 'A_wo': _d[2], 'B_w_gate': _d[3], 'B_w_up': _d[4], 'B_w_down': _d[5], **_const})
    _out, _vjp = jax.vjp(_f, A_x, A_wqkv, A_wo, B_w_gate, B_w_up, B_w_down)
    _grads = _vjp(grad_out)
    _out0 = jnp.asarray(_out)
    return (_out0, *[jnp.asarray(_g) for _g in _grads])
```

```python
import functools

import jax
import jax.numpy as jnp
import jax.experimental.pallas as pl
import jax.experimental.pallas.tpu as pltpu

S = 2048
D = 512
H = 32
DH = 16
W = 256
F = 1376
EPS = 1e-5
TM = 256
NB = S // TM
QB = 128
NSUB = TM // QB
NKEY = W + QB
NG = 4
NEG = -1e9

_NN = (((1,), (0,)), ((), ()))
_NT = (((1,), (1,)), ((), ()))
_TN = (((0,), (0,)), ((), ()))


def _dot(a, b, dims=_NN):
    return jax.lax.dot_general(a, b, dims, preferred_element_type=jnp.float32)


def _ln(x):
    m = jnp.mean(x, axis=-1, keepdims=True)
    xc = x - m
    v = jnp.mean(xc * xc, axis=-1, keepdims=True)
    r = jax.lax.rsqrt(v + EPS)
    return xc * r, r


def _ln_bwd(dy, y, r):
    m1 = jnp.mean(dy, axis=-1, keepdims=True)
    m2 = jnp.mean(dy * y, axis=-1, keepdims=True)
    return r * (dy - m1 - y * m2)


def _kernel(x_ref, xl_ref, dout_ref, wqkv_ref, wo_ref, wg_ref, wu_ref, wd_ref,
            out_ref, dx_ref, dwqkv_ref, dwo_ref, dwg_ref, dwu_ref, dwd_ref,
            q_s, k_s, v_s, kT_s, vT_s, do_s, pT_s, oT_s, dqT_s,
            dk_s, dv_s, dq_s, dh_s,
            aqkv, ao, ag, au, ad):
    i = pl.program_id(0)

    @pl.when(i == 0)
    def _init():
        k_s[:, 0:W, :] = jnp.zeros((NG, W, 128), jnp.bfloat16)
        v_s[:, 0:W, :] = jnp.zeros((NG, W, 128), jnp.bfloat16)
        kT_s[:, 0:W] = jnp.zeros((D, W), jnp.bfloat16)
        vT_s[:, 0:W] = jnp.zeros((D, W), jnp.bfloat16)
        dk_s[...] = jnp.zeros(dk_s.shape, jnp.float32)
        dv_s[...] = jnp.zeros(dv_s.shape, jnp.float32)
        aqkv[...] = jnp.zeros(aqkv.shape, jnp.float32)
        ao[...] = jnp.zeros(ao.shape, jnp.float32)
        ag[...] = jnp.zeros(ag.shape, jnp.float32)
        au[...] = jnp.zeros(au.shape, jnp.float32)
        ad[...] = jnp.zeros(ad.shape, jnp.float32)

    @pl.when(i < NB)
    def _main():
        row0 = pl.multiple_of(i * TM, TM)
        x = x_ref[...].astype(jnp.float32)
        xn1, _ = _ln(x)
        qkv = _dot(xn1.astype(jnp.bfloat16), wqkv_ref[...])
        qf = (qkv[:, 0:D] * (DH ** -0.5)).astype(jnp.bfloat16)
        kf = qkv[:, D:2 * D]
        vf = qkv[:, 2 * D:3 * D]
        kb = kf.astype(jnp.bfloat16)
        vb = vf.astype(jnp.bfloat16)
        for g in range(NG):
            q_s[g] = qf[:, g * 128:(g + 1) * 128]
            k_s[g, pl.ds(W + row0, TM), :] = kb[:, g * 128:(g + 1) * 128]
            v_s[g, pl.ds(W + row0, TM), :] = vb[:, g * 128:(g + 1) * 128]
        kT_s[:, pl.ds(W + row0, TM)] = kf.T.astype(jnp.bfloat16)
        vT_s[:, pl.ds(W + row0, TM)] = vf.T.astype(jnp.bfloat16)

        lane_head = jax.lax.broadcasted_iota(jnp.int32, (QB, 128), 1) // DH

        def _bias(s0):
            r = jax.lax.broadcasted_iota(jnp.int32, (NKEY, QB), 0)
            c = jax.lax.broadcasted_iota(jnp.int32, (NKEY, QB), 1)
            ok = (r > c) & (r - W <= c) & (r >= W - s0)
            return jnp.where(ok, 0.0, NEG).astype(jnp.float32)

        def att_fwd(b, carry):
            q0 = pl.multiple_of(b * QB, QB)
            s0 = pl.multiple_of(row0 + q0, QB)
            bias = _bias(s0)
            for g in range(NG):
                kw = k_s[g, pl.ds(s0, NKEY), :]
                qg = q_s[g, pl.ds(q0, QB), :]
                for hl in range(8):
                    h = g * 8 + hl
                    wq = jnp.where(lane_head == hl, qg, jnp.zeros_like(qg))
                    sT = _dot(kw, wq, _NT) + bias
                    m = jnp.max(sT, axis=0, keepdims=True)
                    p = jnp.exp(sT - m)
                    l = jnp.sum(p, axis=0, keepdims=True)
                    pb = (p * (1.0 / l)).astype(jnp.bfloat16)
                    pT_s[b * H + h] = pb
                    vTw = vT_s[pl.ds(h * DH, DH), pl.ds(s0, NKEY)]
                    oT_s[pl.ds(h * DH, DH), pl.ds(q0, QB)] = _dot(vTw, pb)
            return carry

        jax.lax.fori_loop(0, NSUB, att_fwd, 0)

        oTb = oT_s[...].astype(jnp.bfloat16)
        ob = oT_s[...].T.astype(jnp.bfloat16)
        h1 = x + _dot(ob, wo_ref[...])
        hn, r2 = _ln(h1)
        hnb = hn.astype(jnp.bfloat16)
        gg = _dot(hnb, wg_ref[...])
        uu = _dot(hnb, wu_ref[...])
        sg = jax.nn.sigmoid(gg)
        act = (sg * uu).astype(jnp.bfloat16)
        out_ref[...] = (h1 + _dot(act, wd_ref[...])).astype(out_ref.dtype)

        dout_b = dout_ref[...]
        dout = dout_b.astype(jnp.float32)
        dact = _dot(dout_b, wd_ref[...], _NT)
        du = (dact * sg).astype(jnp.bfloat16)
        dg = (dact * uu * sg * (1.0 - sg)).astype(jnp.bfloat16)
        ad[...] += _dot(act, dout_b, _TN)
        hnT = hn.T.astype(jnp.bfloat16)
        ag[...] += _dot(hnT, dg)
        au[...] += _dot(hnT, du)
        dhn = _dot(dg, wg_ref[...], _NT) + _dot(du, wu_ref[...], _NT)
        dh = dout + _ln_bwd(dhn, hn, r2)
        slot = i % 2
        dh_s[slot] = dh
        dhb = dh.astype(jnp.bfloat16)
        ao[...] += _dot(oTb, dhb)
        dob = _dot(dhb, wo_ref[...], _NT).astype(jnp.bfloat16)
        for g in range(NG):
            do_s[g] = dob[:, g * 128:(g + 1) * 128]

        def att_bwd(b, carry):
            q0 = pl.multiple_of(b * QB, QB)
            s0 = pl.multiple_of(row0 + q0, QB)
            for g in range(NG):
                vw = v_s[g, pl.ds(s0, NKEY), :]
                qg = q_s[g, pl.ds(q0, QB), :]
                dog = do_s[g, pl.ds(q0, QB), :]
                dv_acc = jnp.zeros((NKEY, 128), jnp.float32)
                dk_acc = jnp.zeros((NKEY, 128), jnp.float32)
                for hl in range(8):
                    h = g * 8 + hl
                    sel = lane_head == hl
                    wq = jnp.where(sel, qg, jnp.zeros_like(qg))
                    wdo = jnp.where(sel, dog, jnp.zeros_like(dog))
                    pb = pT_s[b * H + h]
                    p = pb.astype(jnp.float32)
                    dpT = _dot(vw, wdo, _NT)
                    delta = jnp.sum(p * dpT, axis=0, keepdims=True)
                    dsb = (p * (dpT - delta)).astype(jnp.bfloat16)
                    dv_acc = dv_acc + _dot(pb, wdo)
                    dk_acc = dk_acc + _dot(dsb, wq)
                    kTw = kT_s[pl.ds(h * DH, DH), pl.ds(s0, NKEY)]
                    dqT_s[pl.ds(h * DH, DH), pl.ds(q0, QB)] = _dot(kTw, dsb)
                dv_s[g, pl.ds(s0, NKEY), :] += dv_acc
                dk_s[g, pl.ds(s0, NKEY), :] += dk_acc
            return carry

        jax.lax.fori_loop(0, NSUB, att_bwd, 0)
        dq_s[slot] = dqT_s[...].T * (DH ** -0.5)

    @pl.when(i >= 1)
    def _finalize():
        j = i - 1
        row0 = pl.multiple_of(j * TM, TM)
        slot = j % 2
        x = xl_ref[...].astype(jnp.float32)
        xn1, r1 = _ln(x)
        dqb = dq_s[slot].astype(jnp.bfloat16)
        dkb = jnp.concatenate([dk_s[g, pl.ds(W + row0, TM), :] for g in range(NG)], axis=1).astype(jnp.bfloat16)
        dvb = jnp.concatenate([dv_s[g, pl.ds(W + row0, TM), :] for g in range(NG)], axis=1).astype(jnp.bfloat16)
        dqkv = jnp.concatenate([dqb, dkb, dvb], axis=1)
        aqkv[...] += _dot(xn1.T.astype(jnp.bfloat16), dqkv)
        dxn1 = _dot(dqkv, wqkv_ref[...], _NT)
        dx_ref[...] = (dh_s[slot] + _ln_bwd(dxn1, xn1, r1)).astype(dx_ref.dtype)

    @pl.when(i == NB)
    def _write():
        dwqkv_ref[...] = aqkv[...].astype(dwqkv_ref.dtype)
        dwo_ref[...] = ao[...].astype(dwo_ref.dtype)
        dwg_ref[...] = ag[...].astype(dwg_ref.dtype)
        dwu_ref[...] = au[...].astype(dwu_ref.dtype)
        dwd_ref[...] = ad[...].astype(dwd_ref.dtype)


@jax.jit
def pallas_sequential_preLN__sliding_block__glu_gated_glu__prompt_kernel(
    A_x: jax.Array,
    A_wqkv: jax.Array,
    A_wo: jax.Array,
    B_x: jax.Array,
    B_w_gate: jax.Array,
    B_w_up: jax.Array,
    B_w_down: jax.Array,
    grad_out: jax.Array,
):
    del B_x
    x2 = A_x.reshape(S, D)
    g2 = grad_out.reshape(S, D)
    bf = jnp.bfloat16
    f32 = jnp.float32

    cur = lambda i: (jnp.minimum(i, NB - 1), 0)
    lag = lambda i: (jnp.maximum(i - 1, 0), 0)
    const = lambda i: (0, 0)

    def wspec(shape):
        return pl.BlockSpec(shape, const, pipeline_mode=pl.Buffered(1))

    in_specs = [
        pl.BlockSpec((TM, D), cur),
        pl.BlockSpec((TM, D), lag),
        pl.BlockSpec((TM, D), cur),
        wspec((D, 3 * D)), wspec((D, D)), wspec((D, F)), wspec((D, F)), wspec((F, D)),
    ]
    out_specs = [
        pl.BlockSpec((TM, D), cur),
        pl.BlockSpec((TM, D), lag),
        wspec((D, 3 * D)), wspec((D, D)), wspec((D, F)), wspec((D, F)), wspec((F, D)),
    ]
    out_shape = [
        jax.ShapeDtypeStruct((S, D), bf),
        jax.ShapeDtypeStruct((S, D), bf),
        jax.ShapeDtypeStruct((D, 3 * D), bf),
        jax.ShapeDtypeStruct((D, D), bf),
        jax.ShapeDtypeStruct((D, F), bf),
        jax.ShapeDtypeStruct((D, F), bf),
        jax.ShapeDtypeStruct((F, D), bf),
    ]
    scratch = [
        pltpu.VMEM((NG, TM, 128), bf),
        pltpu.VMEM((NG, W + S, 128), bf),
        pltpu.VMEM((NG, W + S, 128), bf),
        pltpu.VMEM((D, W + S), bf),
        pltpu.VMEM((D, W + S), bf),
        pltpu.VMEM((NG, TM, 128), bf),
        pltpu.VMEM((NSUB * H, NKEY, QB), bf),
        pltpu.VMEM((D, TM), f32),
        pltpu.VMEM((D, TM), f32),
        pltpu.VMEM((NG, W + S, 128), f32),
        pltpu.VMEM((NG, W + S, 128), f32),
        pltpu.VMEM((2, TM, D), f32),
        pltpu.VMEM((2, TM, D), f32),
        pltpu.VMEM((D, 3 * D), f32),
        pltpu.VMEM((D, D), f32),
        pltpu.VMEM((D, F), f32),
        pltpu.VMEM((D, F), f32),
        pltpu.VMEM((F, D), f32),
    ]
    outs = pl.pallas_call(
        _kernel,
        grid=(NB + 1,),
        in_specs=in_specs,
        out_specs=out_specs,
        out_shape=out_shape,
        scratch_shapes=scratch,
        compiler_params=pltpu.CompilerParams(
            dimension_semantics=("arbitrary",),
            vmem_limit_bytes=100 * 1024 * 1024,
        ),
    )(x2, x2, g2, A_wqkv, A_wo, B_w_gate, B_w_up, B_w_down)
    out, dx, dwqkv, dwo, dwg, dwu, dwd = outs
    return (out.reshape(1, S, D), dx.reshape(1, S, D), dwqkv, dwo, dwg, dwu, dwd)
```

```python
import functools

import jax
import jax.numpy as jnp
import jax.experimental.pallas as pl
import jax.experimental.pallas.tpu as pltpu

S = 2048
D = 512
H = 32
DH = 16
W = 256
F = 1376
EPS = 1e-5
TM = 256
NB = S // TM
QB = 128
NSUB = TM // QB
NKEY = W + QB
NG = 4
NEG = -1e9
LOG2E = 1.4426950408889634
LN2 = 0.6931471805599453

_NN = (((1,), (0,)), ((), ()))
_NT = (((1,), (1,)), ((), ()))
_TN = (((0,), (0,)), ((), ()))


def _dot(a, b, dims=_NN):
    return jax.lax.dot_general(a, b, dims, preferred_element_type=jnp.float32)


def _ln(x):
    m = jnp.mean(x, axis=-1, keepdims=True)
    xc = x - m
    v = jnp.mean(xc * xc, axis=-1, keepdims=True)
    r = jax.lax.rsqrt(v + EPS)
    return xc * r, r


def _ln_bwd(dy, y, r):
    m1 = jnp.mean(dy, axis=-1, keepdims=True)
    m2 = jnp.mean(dy * y, axis=-1, keepdims=True)
    return r * (dy - m1 - y * m2)


def _col_reduce(x, op, red):
    parts = [x[r * 8:(r + 1) * 8] for r in range(x.shape[0] // 8)]
    while len(parts) > 1:
        nxt = [op(parts[2 * k], parts[2 * k + 1]) for k in range(len(parts) // 2)]
        if len(parts) % 2:
            nxt.append(parts[-1])
        parts = nxt
    return red(parts[0], axis=0, keepdims=True)


def _head_w(slab, hl):
    pieces = []
    if hl > 0:
        pieces.append(jnp.zeros((hl * DH, 128), slab.dtype))
    pieces.append(slab)
    if hl < 7:
        pieces.append(jnp.zeros(((7 - hl) * DH, 128), slab.dtype))
    return jnp.concatenate(pieces, axis=0)


def _kernel(x_ref, xl_ref, dout_ref, wqkv_ref, wo_ref, wg_ref, wu_ref, wd_ref,
            out_ref, dx_ref, dwqkv_ref, dwo_ref, dwg_ref, dwu_ref, dwd_ref,
            qT_s, k_s, v_s, kT_s, vT_s, doT_s, p_s, ds_s, rl_s, oT_s, dqT_s, s_s, m_s,
            dk_s, dv_s, dq_s, dh_s,
            aqkv, ao, ag, au, ad):
    i = pl.program_id(0)

    @pl.when(i == 0)
    def _init():
        k_s[:, 0:W, :] = jnp.zeros((NG, W, 128), jnp.bfloat16)
        v_s[:, 0:W, :] = jnp.zeros((NG, W, 128), jnp.bfloat16)
        kT_s[:, 0:W] = jnp.zeros((D, W), jnp.bfloat16)
        vT_s[:, 0:W] = jnp.zeros((D, W), jnp.bfloat16)
        dk_s[...] = jnp.zeros(dk_s.shape, jnp.float32)
        dv_s[...] = jnp.zeros(dv_s.shape, jnp.float32)
        aqkv[...] = jnp.zeros(aqkv.shape, jnp.float32)
        ao[...] = jnp.zeros(ao.shape, jnp.float32)
        ag[...] = jnp.zeros(ag.shape, jnp.float32)
        au[...] = jnp.zeros(au.shape, jnp.float32)
        ad[...] = jnp.zeros(ad.shape, jnp.float32)

    @pl.when(i < NB)
    def _main():
        row0 = pl.multiple_of(i * TM, TM)
        with jax.named_scope("qkv"):
            x = x_ref[...].astype(jnp.float32)
            xn1, _ = _ln(x)
            qkv = _dot(xn1.astype(jnp.bfloat16), wqkv_ref[...])
            qkvT = qkv.T
            qT_s[...] = (qkvT[0:D] * (DH ** -0.5 * LOG2E)).astype(jnp.bfloat16)
            kT_s[:, pl.ds(W + row0, TM)] = qkvT[D:2 * D].astype(jnp.bfloat16)
            vT_s[:, pl.ds(W + row0, TM)] = qkvT[2 * D:3 * D].astype(jnp.bfloat16)
            kb = qkv[:, D:2 * D].astype(jnp.bfloat16)
            vb = qkv[:, 2 * D:3 * D].astype(jnp.bfloat16)
            for g in range(NG):
                k_s[g, pl.ds(W + row0, TM), :] = kb[:, g * 128:(g + 1) * 128]
                v_s[g, pl.ds(W + row0, TM), :] = vb[:, g * 128:(g + 1) * 128]

        def _bias(s0):
            r = jax.lax.broadcasted_iota(jnp.int32, (NKEY, QB), 0)
            c = jax.lax.broadcasted_iota(jnp.int32, (NKEY, QB), 1)
            ok = (r > c) & (r - W <= c) & (r >= W - s0)
            return jnp.where(ok, 0.0, NEG).astype(jnp.float32)

        def att_fwd(b, carry):
            q0 = pl.multiple_of(b * QB, QB)
            s0 = pl.multiple_of(row0 + q0, QB)
            bias = _bias(s0)
            for g in range(NG):
                kw = k_s[g, pl.ds(s0, NKEY), :]
                for hl in range(8):
                    h = g * 8 + hl
                    wq = _head_w(qT_s[pl.ds(h * DH, DH), pl.ds(q0, QB)], hl)
                    sT = _dot(kw, wq) + bias
                    s_s[g, :, hl * 128:(hl + 1) * 128] = sT
                    m_s[h:h + 1, :] = _col_reduce(sT, jnp.maximum, jnp.max)
            for g in range(NG):
                for hl in range(8):
                    h = g * 8 + hl
                    p = jnp.exp2(s_s[g, :, hl * 128:(hl + 1) * 128] - m_s[h:h + 1, :])
                    l = _col_reduce(p, jnp.add, jnp.sum)
                    p_s[b, g, :, hl * 128:(hl + 1) * 128] = p.astype(jnp.bfloat16)
                    rl_s[b, h:h + 1, :] = 1.0 / l
            for g in range(NG):
                for hl in range(8):
                    h = g * 8 + hl
                    vTw = vT_s[pl.ds(h * DH, DH), pl.ds(s0, NKEY)]
                    oT_s[pl.ds(h * DH, DH), pl.ds(q0, QB)] = (
                        _dot(vTw, p_s[b, g, :, hl * 128:(hl + 1) * 128]) * rl_s[b, h:h + 1, :])
            return carry

        with jax.named_scope("att_fwd"):
            jax.lax.fori_loop(0, NSUB, att_fwd, 0)

        with jax.named_scope("mlp_fwd"):
            oTb = oT_s[...].astype(jnp.bfloat16)
            h1 = x + _dot(oTb, wo_ref[...], _TN)
            hn, r2 = _ln(h1)
            hnb = hn.astype(jnp.bfloat16)
            gg = _dot(hnb, wg_ref[...])
            uu = _dot(hnb, wu_ref[...])
            sg = jax.nn.sigmoid(gg)
            act = (sg * uu).astype(jnp.bfloat16)
            out_ref[...] = (h1 + _dot(act, wd_ref[...])).astype(out_ref.dtype)

        with jax.named_scope("mlp_bwd"):
            dout_b = dout_ref[...]
            dout = dout_b.astype(jnp.float32)
            dact = _dot(dout_b, wd_ref[...], _NT)
            du = (dact * sg).astype(jnp.bfloat16)
            dg = (dact * uu * sg * (1.0 - sg)).astype(jnp.bfloat16)
            ad[...] += _dot(act, dout_b, _TN)
            hnT = hn.T.astype(jnp.bfloat16)
            ag[...] += _dot(hnT, dg)
            au[...] += _dot(hnT, du)
            dhn = _dot(dg, wg_ref[...], _NT) + _dot(du, wu_ref[...], _NT)
            dh = dout + _ln_bwd(dhn, hn, r2)
            slot = i % 2
            dh_s[slot] = dh
            dhb = dh.astype(jnp.bfloat16)
            ao[...] += _dot(oTb, dhb)
            doT_s[...] = _dot(wo_ref[...], dhb, _NT)

        def att_bwd(b, carry):
            q0 = pl.multiple_of(b * QB, QB)
            s0 = pl.multiple_of(row0 + q0, QB)

            def wdo(g, hl):
                h = g * 8 + hl
                slab = (doT_s[pl.ds(h * DH, DH), pl.ds(q0, QB)] * rl_s[b, h:h + 1, :]).astype(jnp.bfloat16)
                return _head_w(slab, hl)

            def wq(g, hl):
                h = g * 8 + hl
                return _head_w(qT_s[pl.ds(h * DH, DH), pl.ds(q0, QB)], hl)

            for g in range(NG):
                vw = v_s[g, pl.ds(s0, NKEY), :]
                for hl in range(8):
                    h = g * 8 + hl
                    dpT = _dot(vw, wdo(g, hl))
                    s_s[g, :, hl * 128:(hl + 1) * 128] = dpT
                    p = p_s[b, g, :, hl * 128:(hl + 1) * 128].astype(jnp.float32)
                    m_s[h:h + 1, :] = _col_reduce(p * dpT, jnp.add, jnp.sum) * rl_s[b, h:h + 1, :]
            for g in range(NG):
                wdo_all = jnp.concatenate([wdo(g, hl) for hl in range(8)], axis=1)
                dv_s[g, pl.ds(s0, NKEY), :] += _dot(p_s[b, g], wdo_all, _NT)
            for g in range(NG):
                for hl in range(8):
                    h = g * 8 + hl
                    p = p_s[b, g, :, hl * 128:(hl + 1) * 128].astype(jnp.float32)
                    ds_s[g, :, hl * 128:(hl + 1) * 128] = (
                        p * (s_s[g, :, hl * 128:(hl + 1) * 128] - m_s[h:h + 1, :])).astype(jnp.bfloat16)
            for g in range(NG):
                for hl in range(8):
                    h = g * 8 + hl
                    kTw = kT_s[pl.ds(h * DH, DH), pl.ds(s0, NKEY)]
                    dqT_s[pl.ds(h * DH, DH), pl.ds(q0, QB)] = _dot(kTw, ds_s[g, :, hl * 128:(hl + 1) * 128])
            for g in range(NG):
                wq_all = jnp.concatenate([wq(g, hl) for hl in range(8)], axis=1)
                dk_s[g, pl.ds(s0, NKEY), :] += _dot(ds_s[g], wq_all, _NT)
            return carry

        with jax.named_scope("att_bwd"):
            jax.lax.fori_loop(0, NSUB, att_bwd, 0)
            dq_s[slot] = dqT_s[...].T * (DH ** -0.5)

    @pl.when(i >= 1)
    def _finalize():
        with jax.named_scope("finalize"):
            j = i - 1
            row0 = pl.multiple_of(j * TM, TM)
            slot = j % 2
            x = xl_ref[...].astype(jnp.float32)
            xn1, r1 = _ln(x)
            dqb = dq_s[slot].astype(jnp.bfloat16)
            dkb = (jnp.concatenate([dk_s[g, pl.ds(W + row0, TM), :] for g in range(NG)], axis=1) * LN2).astype(jnp.bfloat16)
            dvb = jnp.concatenate([dv_s[g, pl.ds(W + row0, TM), :] for g in range(NG)], axis=1).astype(jnp.bfloat16)
            dqkv = jnp.concatenate([dqb, dkb, dvb], axis=1)
            aqkv[...] += _dot(xn1.T.astype(jnp.bfloat16), dqkv)
            dxn1 = _dot(dqkv, wqkv_ref[...], _NT)
            dx_ref[...] = (dh_s[slot] + _ln_bwd(dxn1, xn1, r1)).astype(dx_ref.dtype)

    @pl.when(i == NB)
    def _write():
        dwqkv_ref[...] = aqkv[...].astype(dwqkv_ref.dtype)
        dwo_ref[...] = ao[...].astype(dwo_ref.dtype)
        dwg_ref[...] = ag[...].astype(dwg_ref.dtype)
        dwu_ref[...] = au[...].astype(dwu_ref.dtype)
        dwd_ref[...] = ad[...].astype(dwd_ref.dtype)


@jax.jit
def pallas_sequential_preLN__sliding_block__glu_gated_glu__prompt_kernel(
    A_x: jax.Array,
    A_wqkv: jax.Array,
    A_wo: jax.Array,
    B_x: jax.Array,
    B_w_gate: jax.Array,
    B_w_up: jax.Array,
    B_w_down: jax.Array,
    grad_out: jax.Array,
):
    del B_x
    x2 = A_x.reshape(S, D)
    g2 = grad_out.reshape(S, D)
    bf = jnp.bfloat16
    f32 = jnp.float32

    cur = lambda i: (jnp.minimum(i, NB - 1), 0)
    lag = lambda i: (jnp.maximum(i - 1, 0), 0)
    const = lambda i: (0, 0)

    def wspec(shape):
        return pl.BlockSpec(shape, const, pipeline_mode=pl.Buffered(1))

    in_specs = [
        pl.BlockSpec((TM, D), cur),
        pl.BlockSpec((TM, D), lag),
        pl.BlockSpec((TM, D), cur),
        wspec((D, 3 * D)), wspec((D, D)), wspec((D, F)), wspec((D, F)), wspec((F, D)),
    ]
    out_specs = [
        pl.BlockSpec((TM, D), cur),
        pl.BlockSpec((TM, D), lag),
        wspec((D, 3 * D)), wspec((D, D)), wspec((D, F)), wspec((D, F)), wspec((F, D)),
    ]
    out_shape = [
        jax.ShapeDtypeStruct((S, D), bf),
        jax.ShapeDtypeStruct((S, D), bf),
        jax.ShapeDtypeStruct((D, 3 * D), bf),
        jax.ShapeDtypeStruct((D, D), bf),
        jax.ShapeDtypeStruct((D, F), bf),
        jax.ShapeDtypeStruct((D, F), bf),
        jax.ShapeDtypeStruct((F, D), bf),
    ]
    scratch = [
        pltpu.VMEM((D, TM), bf),
        pltpu.VMEM((NG, W + S, 128), bf),
        pltpu.VMEM((NG, W + S, 128), bf),
        pltpu.VMEM((D, W + S), bf),
        pltpu.VMEM((D, W + S), bf),
        pltpu.VMEM((D, TM), f32),
        pltpu.VMEM((NSUB, NG, NKEY, 8 * 128), bf),
        pltpu.VMEM((NG, NKEY, 8 * 128), bf),
        pltpu.VMEM((NSUB, H, 128), f32),
        pltpu.VMEM((D, TM), f32),
        pltpu.VMEM((D, TM), f32),
        pltpu.VMEM((NG, NKEY, 8 * 128), f32),
        pltpu.VMEM((H, 128), f32),
        pltpu.VMEM((NG, W + S, 128), f32),
        pltpu.VMEM((NG, W + S, 128), f32),
        pltpu.VMEM((2, TM, D), f32),
        pltpu.VMEM((2, TM, D), f32),
        pltpu.VMEM((D, 3 * D), f32),
        pltpu.VMEM((D, D), f32),
        pltpu.VMEM((D, F), f32),
        pltpu.VMEM((D, F), f32),
        pltpu.VMEM((F, D), f32),
    ]
    outs = pl.pallas_call(
        _kernel,
        grid=(NB + 1,),
        in_specs=in_specs,
        out_specs=out_specs,
        out_shape=out_shape,
        scratch_shapes=scratch,
        compiler_params=pltpu.CompilerParams(
            dimension_semantics=("arbitrary",),
            vmem_limit_bytes=100 * 1024 * 1024,
        ),
    )(x2, x2, g2, A_wqkv, A_wo, B_w_gate, B_w_up, B_w_down)
    out, dx, dwqkv, dwo, dwg, dwu, dwd = outs
    return (out.reshape(1, S, D), dx.reshape(1, S, D), dwqkv, dwo, dwg, dwu, dwd)
```

```python
import functools

import jax
import jax.numpy as jnp
import jax.experimental.pallas as pl
import jax.experimental.pallas.tpu as pltpu

S = 2048
D = 512
H = 32
DH = 16
W = 256
F = 1376
EPS = 1e-5
TM = 256
NB = S // TM
QB = 128
NSUB = TM // QB
NKEY = W + QB
NG = 4
NEG = -1e9
LOG2E = 1.4426950408889634
LN2 = 0.6931471805599453

_NN = (((1,), (0,)), ((), ()))
_NT = (((1,), (1,)), ((), ()))
_TN = (((0,), (0,)), ((), ()))


def _dot(a, b, dims=_NN):
    return jax.lax.dot_general(a, b, dims, preferred_element_type=jnp.float32)


def _ln(x):
    m = jnp.mean(x, axis=-1, keepdims=True)
    xc = x - m
    v = jnp.mean(xc * xc, axis=-1, keepdims=True)
    r = jax.lax.rsqrt(v + EPS)
    return xc * r, r


def _ln_bwd(dy, y, r):
    m1 = jnp.mean(dy, axis=-1, keepdims=True)
    m2 = jnp.mean(dy * y, axis=-1, keepdims=True)
    return r * (dy - m1 - y * m2)


def _col_reduce(x, op, red):
    parts = [x[r * 8:(r + 1) * 8] for r in range(x.shape[0] // 8)]
    while len(parts) > 1:
        nxt = [op(parts[2 * k], parts[2 * k + 1]) for k in range(len(parts) // 2)]
        if len(parts) % 2:
            nxt.append(parts[-1])
        parts = nxt
    return red(parts[0], axis=0, keepdims=True)


def _head_w(slab, hl):
    pieces = []
    if hl > 0:
        pieces.append(jnp.zeros((hl * DH, 128), slab.dtype))
    pieces.append(slab)
    if hl < 7:
        pieces.append(jnp.zeros(((7 - hl) * DH, 128), slab.dtype))
    return jnp.concatenate(pieces, axis=0)


def _kernel(x_ref, xl_ref, dout_ref, wqkv_h, wo_h, wg_h, wu_h, wd_h,
            out_ref, dx_ref, dwqkv_h, dwo_h, dwg_h, dwu_h, dwd_h,
            wqkv_ref, wo_ref, wg_ref, wu_ref, wd_ref,
            dwqkv_ref, dwo_ref, dwg_ref, dwu_ref, dwd_ref, sem_in, sem_out,
            qT_s, k_s, v_s, kT_s, vT_s, doT_s, p_s, ds_s, rl_s, oT_s, dqT_s, s_s, m_s,
            dkT_s, dvT_s, dq_s, dh_s,
            aqkv, ao, ag, au, ad):
    i = pl.program_id(0)

    w_src = (wqkv_h, wo_h, wg_h, wu_h, wd_h)
    w_dst = (wqkv_ref, wo_ref, wg_ref, wu_ref, wd_ref)
    g_src = (dwqkv_ref, dwo_ref, dwg_ref, dwu_ref, dwd_ref)
    g_dst = (dwqkv_h, dwo_h, dwg_h, dwu_h, dwd_h)

    def in_copy(k):
        return pltpu.make_async_copy(w_src[k], w_dst[k], sem_in.at[k])

    def out_copy(k):
        return pltpu.make_async_copy(g_src[k], g_dst[k], sem_out.at[k])

    @pl.when(i == 0)
    def _init():
        for k in range(5):
            in_copy(k).start()
        k_s[:, 0:W, :] = jnp.zeros((NG, W, 128), jnp.bfloat16)
        v_s[:, 0:W, :] = jnp.zeros((NG, W, 128), jnp.bfloat16)
        kT_s[:, 0:W] = jnp.zeros((D, W), jnp.bfloat16)
        vT_s[:, 0:W] = jnp.zeros((D, W), jnp.bfloat16)
        dkT_s[...] = jnp.zeros(dkT_s.shape, jnp.float32)
        dvT_s[...] = jnp.zeros(dvT_s.shape, jnp.float32)
        aqkv[...] = jnp.zeros(aqkv.shape, jnp.float32)
        ao[...] = jnp.zeros(ao.shape, jnp.float32)
        ag[...] = jnp.zeros(ag.shape, jnp.float32)
        au[...] = jnp.zeros(au.shape, jnp.float32)
        ad[...] = jnp.zeros(ad.shape, jnp.float32)
        in_copy(0).wait()

    @pl.when(i < NB)
    def _main():
        row0 = pl.multiple_of(i * TM, TM)
        with jax.named_scope("qkv"):
            x = x_ref[...].astype(jnp.float32)
            xn1, _ = _ln(x)
            qkv = _dot(xn1.astype(jnp.bfloat16), wqkv_ref[...])
            qkvT = qkv.T
            qT_s[...] = (qkvT[0:D] * (DH ** -0.5 * LOG2E)).astype(jnp.bfloat16)
            kT_s[:, pl.ds(W + row0, TM)] = qkvT[D:2 * D].astype(jnp.bfloat16)
            vT_s[:, pl.ds(W + row0, TM)] = qkvT[2 * D:3 * D].astype(jnp.bfloat16)
            kb = qkv[:, D:2 * D].astype(jnp.bfloat16)
            vb = qkv[:, 2 * D:3 * D].astype(jnp.bfloat16)
            for g in range(NG):
                k_s[g, pl.ds(W + row0, TM), :] = kb[:, g * 128:(g + 1) * 128]
                v_s[g, pl.ds(W + row0, TM), :] = vb[:, g * 128:(g + 1) * 128]

        def _bias(s0):
            r = jax.lax.broadcasted_iota(jnp.int32, (NKEY, QB), 0)
            c = jax.lax.broadcasted_iota(jnp.int32, (NKEY, QB), 1)
            ok = (r > c) & (r - W <= c) & (r >= W - s0)
            return jnp.where(ok, 0.0, NEG).astype(jnp.float32)

        def att_fwd(b, carry):
            q0 = pl.multiple_of(b * QB, QB)
            s0 = pl.multiple_of(row0 + q0, QB)
            bias = _bias(s0)
            for g in range(NG):
                kw = k_s[g, pl.ds(s0, NKEY), :]
                for hl in range(8):
                    h = g * 8 + hl
                    wq = _head_w(qT_s[pl.ds(h * DH, DH), pl.ds(q0, QB)], hl)
                    sT = _dot(kw, wq) + bias
                    s_s[g, :, hl * 128:(hl + 1) * 128] = sT
                    m_s[h:h + 1, :] = _col_reduce(sT, jnp.maximum, jnp.max)
            for g in range(NG):
                for hl in range(8):
                    h = g * 8 + hl
                    p = jnp.exp2(s_s[g, :, hl * 128:(hl + 1) * 128] - m_s[h:h + 1, :])
                    l = _col_reduce(p, jnp.add, jnp.sum)
                    p_s[b, g, :, hl * 128:(hl + 1) * 128] = p.astype(jnp.bfloat16)
                    rl_s[b, h:h + 1, :] = 1.0 / l
            for g in range(NG):
                for hl in range(8):
                    h = g * 8 + hl
                    vTw = vT_s[pl.ds(h * DH, DH), pl.ds(s0, NKEY)]
                    oT_s[pl.ds(h * DH, DH), pl.ds(q0, QB)] = (
                        _dot(vTw, p_s[b, g, :, hl * 128:(hl + 1) * 128]) * rl_s[b, h:h + 1, :])
            return carry

        with jax.named_scope("att_fwd"):
            jax.lax.fori_loop(0, NSUB, att_fwd, 0)

        @pl.when(i == 0)
        def _wait_w():
            for k in range(1, 5):
                in_copy(k).wait()

        with jax.named_scope("mlp_fwd"):
            oTb = oT_s[...].astype(jnp.bfloat16)
            h1 = x + _dot(oTb, wo_ref[...], _TN)
            hn, r2 = _ln(h1)
            hnb = hn.astype(jnp.bfloat16)
            gg = _dot(hnb, wg_ref[...], _NT)
            uu = _dot(hnb, wu_ref[...], _NT)
            sg = jax.nn.sigmoid(gg)
            act = (sg * uu).astype(jnp.bfloat16)
            out_ref[...] = (h1 + _dot(act, wd_ref[...])).astype(out_ref.dtype)

        with jax.named_scope("mlp_bwd"):
            dout_b = dout_ref[...]
            dout = dout_b.astype(jnp.float32)
            dact = _dot(dout_b, wd_ref[...], _NT)
            du = (dact * sg).astype(jnp.bfloat16)
            dg = (dact * uu * sg * (1.0 - sg)).astype(jnp.bfloat16)
            ad[...] += _dot(act, dout_b, _TN)
            hnT = hn.T.astype(jnp.bfloat16)
            ag[...] += _dot(hnT, dg)
            au[...] += _dot(hnT, du)
            dhn = _dot(dg, wg_ref[...]) + _dot(du, wu_ref[...])
            dh = dout + _ln_bwd(dhn, hn, r2)
            slot = i % 2
            dh_s[slot] = dh
            dhb = dh.astype(jnp.bfloat16)
            ao[...] += _dot(oTb, dhb)
            doT_s[...] = _dot(wo_ref[...], dhb, _NT)

        @pl.when(i == NB - 1)
        def _write_mlp_grads():
            dwo_ref[...] = ao[...].astype(dwo_ref.dtype)
            dwg_ref[...] = ag[...].T.astype(dwg_ref.dtype)
            dwu_ref[...] = au[...].T.astype(dwu_ref.dtype)
            dwd_ref[...] = ad[...].astype(dwd_ref.dtype)
            for k in range(1, 5):
                out_copy(k).start()

        def att_bwd(b, carry):
            q0 = pl.multiple_of(b * QB, QB)
            s0 = pl.multiple_of(row0 + q0, QB)

            def wdo(g, hl):
                h = g * 8 + hl
                slab = (doT_s[pl.ds(h * DH, DH), pl.ds(q0, QB)] * rl_s[b, h:h + 1, :]).astype(jnp.bfloat16)
                return _head_w(slab, hl)

            def wq(g, hl):
                h = g * 8 + hl
                return _head_w(qT_s[pl.ds(h * DH, DH), pl.ds(q0, QB)], hl)

            for g in range(NG):
                vw = v_s[g, pl.ds(s0, NKEY), :]
                for hl in range(8):
                    h = g * 8 + hl
                    dpT = _dot(vw, wdo(g, hl))
                    s_s[g, :, hl * 128:(hl + 1) * 128] = dpT
                    p = p_s[b, g, :, hl * 128:(hl + 1) * 128].astype(jnp.float32)
                    m_s[h:h + 1, :] = _col_reduce(p * dpT, jnp.add, jnp.sum) * rl_s[b, h:h + 1, :]
            for g in range(NG):
                for hl in range(8):
                    h = g * 8 + hl
                    slab = (doT_s[pl.ds(h * DH, DH), pl.ds(q0, QB)] * rl_s[b, h:h + 1, :]).astype(jnp.bfloat16)
                    dvT_s[pl.ds(h * DH, DH), pl.ds(s0, NKEY)] += _dot(
                        slab, p_s[b, g, :, hl * 128:(hl + 1) * 128], _NT)
            for g in range(NG):
                for hl in range(8):
                    h = g * 8 + hl
                    p = p_s[b, g, :, hl * 128:(hl + 1) * 128].astype(jnp.float32)
                    ds_s[g, :, hl * 128:(hl + 1) * 128] = (
                        p * (s_s[g, :, hl * 128:(hl + 1) * 128] - m_s[h:h + 1, :])).astype(jnp.bfloat16)
            for g in range(NG):
                for hl in range(8):
                    h = g * 8 + hl
                    kTw = kT_s[pl.ds(h * DH, DH), pl.ds(s0, NKEY)]
                    dqT_s[pl.ds(h * DH, DH), pl.ds(q0, QB)] = _dot(kTw, ds_s[g, :, hl * 128:(hl + 1) * 128])
            for g in range(NG):
                for hl in range(8):
                    h = g * 8 + hl
                    dkT_s[pl.ds(h * DH, DH), pl.ds(s0, NKEY)] += _dot(
                        qT_s[pl.ds(h * DH, DH), pl.ds(q0, QB)], ds_s[g, :, hl * 128:(hl + 1) * 128], _NT)
            return carry

        with jax.named_scope("att_bwd"):
            jax.lax.fori_loop(0, NSUB, att_bwd, 0)
            dq_s[slot] = dqT_s[...] * (DH ** -0.5)

    @pl.when(i >= 1)
    def _finalize():
        with jax.named_scope("finalize"):
            j = i - 1
            row0 = pl.multiple_of(j * TM, TM)
            slot = j % 2
            x = xl_ref[...].astype(jnp.float32)
            xn1, r1 = _ln(x)
            dqkvT = jnp.concatenate([
                dq_s[slot].astype(jnp.bfloat16),
                (dkT_s[:, pl.ds(W + row0, TM)] * LN2).astype(jnp.bfloat16),
                dvT_s[:, pl.ds(W + row0, TM)].astype(jnp.bfloat16)], axis=0)
            aqkv[...] += _dot(dqkvT, xn1.astype(jnp.bfloat16))
            dxn1 = _dot(wqkv_ref[...], dqkvT).T
            dx_ref[...] = (dh_s[slot] + _ln_bwd(dxn1, xn1, r1)).astype(dx_ref.dtype)

    @pl.when(i == NB)
    def _write():
        dwqkv_ref[...] = aqkv[...].T.astype(dwqkv_ref.dtype)
        out_copy(0).start()
        for k in range(5):
            out_copy(k).wait()


@jax.jit
def pallas_sequential_preLN__sliding_block__glu_gated_glu__prompt_kernel(
    A_x: jax.Array,
    A_wqkv: jax.Array,
    A_wo: jax.Array,
    B_x: jax.Array,
    B_w_gate: jax.Array,
    B_w_up: jax.Array,
    B_w_down: jax.Array,
    grad_out: jax.Array,
):
    del B_x
    x2 = A_x.reshape(S, D)
    g2 = grad_out.reshape(S, D)
    bf = jnp.bfloat16
    f32 = jnp.float32

    cur = lambda i: (jnp.minimum(i, NB - 1), 0)
    lag = lambda i: (jnp.maximum(i - 1, 0), 0)
    const = lambda i: (0, 0)

    def wspec(shape):
        return pl.BlockSpec(shape, const, pipeline_mode=pl.Buffered(1))

    in_specs = [
        pl.BlockSpec((TM, D), cur),
        pl.BlockSpec((TM, D), lag),
        pl.BlockSpec((TM, D), cur),
    ] + [pl.BlockSpec(memory_space=pl.ANY)] * 5
    out_specs = [
        pl.BlockSpec((TM, D), cur),
        pl.BlockSpec((TM, D), lag),
    ] + [pl.BlockSpec(memory_space=pl.ANY)] * 5
    out_shape = [
        jax.ShapeDtypeStruct((S, D), bf),
        jax.ShapeDtypeStruct((S, D), bf),
        jax.ShapeDtypeStruct((D, 3 * D), bf),
        jax.ShapeDtypeStruct((D, D), bf),
        jax.ShapeDtypeStruct((F, D), bf),
        jax.ShapeDtypeStruct((F, D), bf),
        jax.ShapeDtypeStruct((F, D), bf),
    ]
    wshapes = [(D, 3 * D), (D, D), (F, D), (F, D), (F, D)]
    scratch = [pltpu.VMEM(sh, bf) for sh in wshapes] + [pltpu.VMEM(sh, bf) for sh in wshapes] + [
        pltpu.SemaphoreType.DMA((5,)),
        pltpu.SemaphoreType.DMA((5,)),
        pltpu.VMEM((D, TM), bf),
        pltpu.VMEM((NG, W + S, 128), bf),
        pltpu.VMEM((NG, W + S, 128), bf),
        pltpu.VMEM((D, W + S), bf),
        pltpu.VMEM((D, W + S), bf),
        pltpu.VMEM((D, TM), f32),
        pltpu.VMEM((NSUB, NG, NKEY, 8 * 128), bf),
        pltpu.VMEM((NG, NKEY, 8 * 128), bf),
        pltpu.VMEM((NSUB, H, 128), f32),
        pltpu.VMEM((D, TM), f32),
        pltpu.VMEM((D, TM), f32),
        pltpu.VMEM((NG, NKEY, 8 * 128), f32),
        pltpu.VMEM((H, 128), f32),
        pltpu.VMEM((D, W + S), f32),
        pltpu.VMEM((D, W + S), f32),
        pltpu.VMEM((2, D, TM), f32),
        pltpu.VMEM((2, TM, D), f32),
        pltpu.VMEM((3 * D, D), f32),
        pltpu.VMEM((D, D), f32),
        pltpu.VMEM((D, F), f32),
        pltpu.VMEM((D, F), f32),
        pltpu.VMEM((F, D), f32),
    ]
    outs = pl.pallas_call(
        _kernel,
        grid=(NB + 1,),
        in_specs=in_specs,
        out_specs=out_specs,
        out_shape=out_shape,
        scratch_shapes=scratch,
        compiler_params=pltpu.CompilerParams(
            dimension_semantics=("arbitrary",),
            vmem_limit_bytes=100 * 1024 * 1024,
        ),
    )(x2, x2, g2, A_wqkv, A_wo, B_w_gate.T, B_w_up.T, B_w_down)
    out, dx, dwqkv, dwo, dwg, dwu, dwd = outs
    return (out.reshape(1, S, D), dx.reshape(1, S, D), dwqkv, dwo, dwg.T, dwu.T, dwd)
```

```python
import functools

import jax
import jax.numpy as jnp
import jax.experimental.pallas as pl
import jax.experimental.pallas.tpu as pltpu

S = 2048
D = 512
H = 32
DH = 16
W = 256
F = 1376
EPS = 1e-5
TM = 256
NB = S // TM
QB = 128
NSUB = TM // QB
NKEY = W + QB
NG = 4
NEG = -1e9
LOG2E = 1.4426950408889634
LN2 = 0.6931471805599453

_NN = (((1,), (0,)), ((), ()))
_NT = (((1,), (1,)), ((), ()))
_TN = (((0,), (0,)), ((), ()))


def _dot(a, b, dims=_NN):
    return jax.lax.dot_general(a, b, dims, preferred_element_type=jnp.float32)


def _ln(x):
    m = jnp.mean(x, axis=-1, keepdims=True)
    xc = x - m
    v = jnp.mean(xc * xc, axis=-1, keepdims=True)
    r = jax.lax.rsqrt(v + EPS)
    return xc * r, r


def _ln_bwd(dy, y, r):
    m1 = jnp.mean(dy, axis=-1, keepdims=True)
    m2 = jnp.mean(dy * y, axis=-1, keepdims=True)
    return r * (dy - m1 - y * m2)


def _col_reduce(x, op, red):
    parts = [x[r * 8:(r + 1) * 8] for r in range(x.shape[0] // 8)]
    while len(parts) > 1:
        nxt = [op(parts[2 * k], parts[2 * k + 1]) for k in range(len(parts) // 2)]
        if len(parts) % 2:
            nxt.append(parts[-1])
        parts = nxt
    return red(parts[0], axis=0, keepdims=True)


def _head_w(slab, hl):
    pieces = []
    if hl > 0:
        pieces.append(jnp.zeros((hl * DH, 128), slab.dtype))
    pieces.append(slab)
    if hl < 7:
        pieces.append(jnp.zeros(((7 - hl) * DH, 128), slab.dtype))
    return jnp.concatenate(pieces, axis=0)


def _kernel(x_ref, dout_ref, wqkv_h, wo_h, wg_h, wu_h, wd_h,
            out_ref, dx_ref, dwqkv_h, dwo_h, dwg_h, dwu_h, dwd_h,
            wqkv_ref, wo_ref, wg_ref, wu_ref, wd_ref,
            dwqkv_ref, dwo_ref, dwg_ref, dwu_ref, dwd_ref, sem_in, sem_out,
            qT_s, k_s, v_s, kT_s, vT_s, doT_s, p_s, ds_s, rl_s, oT_s, dqT_s, s_s, m_s,
            dkT_s, dvT_s, dq_s, dh_s, xn_s, r1_s,
            aqkv, ao, ag, au, ad):
    i = pl.program_id(0)

    w_src = (wqkv_h, wo_h, wg_h, wu_h, wd_h)
    w_dst = (wqkv_ref, wo_ref, wg_ref, wu_ref, wd_ref)
    g_src = (dwqkv_ref, dwo_ref, dwg_ref, dwu_ref, dwd_ref)
    g_dst = (dwqkv_h, dwo_h, dwg_h, dwu_h, dwd_h)

    def in_copy(k):
        return pltpu.make_async_copy(w_src[k], w_dst[k], sem_in.at[k])

    def out_copy(k):
        return pltpu.make_async_copy(g_src[k], g_dst[k], sem_out.at[k])

    @pl.when(i == 0)
    def _init():
        for k in range(5):
            in_copy(k).start()
        k_s[:, 0:W, :] = jnp.zeros((NG, W, 128), jnp.bfloat16)
        v_s[:, 0:W, :] = jnp.zeros((NG, W, 128), jnp.bfloat16)
        kT_s[:, 0:W] = jnp.zeros((D, W), jnp.bfloat16)
        vT_s[:, 0:W] = jnp.zeros((D, W), jnp.bfloat16)
        dkT_s[...] = jnp.zeros(dkT_s.shape, jnp.float32)
        dvT_s[...] = jnp.zeros(dvT_s.shape, jnp.float32)
        aqkv[...] = jnp.zeros(aqkv.shape, jnp.float32)
        ao[...] = jnp.zeros(ao.shape, jnp.float32)
        ag[...] = jnp.zeros(ag.shape, jnp.float32)
        au[...] = jnp.zeros(au.shape, jnp.float32)
        ad[...] = jnp.zeros(ad.shape, jnp.float32)
        in_copy(0).wait()

    @pl.when(i < NB)
    def _main():
        row0 = pl.multiple_of(i * TM, TM)
        slot = i % 2
        with jax.named_scope("qkv"):
            x = x_ref[...].astype(jnp.float32)
            xn1, r1 = _ln(x)
            xn_s[slot] = xn1
            r1_s[slot] = r1
            qkv = _dot(xn1.astype(jnp.bfloat16), wqkv_ref[...])
            qkvT = qkv.T
            qT_s[...] = (qkvT[0:D] * (DH ** -0.5 * LOG2E)).astype(jnp.bfloat16)
            kT_s[:, pl.ds(W + row0, TM)] = qkvT[D:2 * D].astype(jnp.bfloat16)
            vT_s[:, pl.ds(W + row0, TM)] = qkvT[2 * D:3 * D].astype(jnp.bfloat16)
            kb = qkv[:, D:2 * D].astype(jnp.bfloat16)
            vb = qkv[:, 2 * D:3 * D].astype(jnp.bfloat16)
            for g in range(NG):
                k_s[g, pl.ds(W + row0, TM), :] = kb[:, g * 128:(g + 1) * 128]
                v_s[g, pl.ds(W + row0, TM), :] = vb[:, g * 128:(g + 1) * 128]

        def _bias(s0):
            r = jax.lax.broadcasted_iota(jnp.int32, (NKEY, QB), 0)
            c = jax.lax.broadcasted_iota(jnp.int32, (NKEY, QB), 1)
            ok = (r > c) & (r - W <= c) & (r >= W - s0)
            return jnp.where(ok, 0.0, NEG).astype(jnp.float32)

        def att_fwd(b, carry):
            q0 = pl.multiple_of(b * QB, QB)
            s0 = pl.multiple_of(row0 + q0, QB)
            bias = _bias(s0)
            for g in range(NG):
                kw = k_s[g, pl.ds(s0, NKEY), :]
                for hl in range(8):
                    h = g * 8 + hl
                    wq = _head_w(qT_s[pl.ds(h * DH, DH), pl.ds(q0, QB)], hl)
                    sT = _dot(kw, wq) + bias
                    s_s[g, :, hl * 128:(hl + 1) * 128] = sT
                    m_s[h:h + 1, :] = _col_reduce(sT, jnp.maximum, jnp.max)
            for g in range(NG):
                for hl in range(8):
                    h = g * 8 + hl
                    p = jnp.exp2(s_s[g, :, hl * 128:(hl + 1) * 128] - m_s[h:h + 1, :])
                    l = _col_reduce(p, jnp.add, jnp.sum)
                    p_s[b, g, :, hl * 128:(hl + 1) * 128] = p.astype(jnp.bfloat16)
                    rl_s[b, h:h + 1, :] = 1.0 / l
            for g in range(NG):
                for hl in range(8):
                    h = g * 8 + hl
                    vTw = vT_s[pl.ds(h * DH, DH), pl.ds(s0, NKEY)]
                    oT_s[pl.ds(h * DH, DH), pl.ds(q0, QB)] = (
                        _dot(vTw, p_s[b, g, :, hl * 128:(hl + 1) * 128]) * rl_s[b, h:h + 1, :])
            return carry

        with jax.named_scope("att_fwd"):
            jax.lax.fori_loop(0, NSUB, att_fwd, 0)

        @pl.when(i == 0)
        def _wait_w():
            for k in range(1, 5):
                in_copy(k).wait()

        with jax.named_scope("mlp_fwd"):
            oTb = oT_s[...].astype(jnp.bfloat16)
            h1 = x + _dot(oTb, wo_ref[...], _TN)
            hn, r2 = _ln(h1)
            hnb = hn.astype(jnp.bfloat16)
            gg = _dot(hnb, wg_ref[...], _NT)
            uu = _dot(hnb, wu_ref[...], _NT)
            sg = jax.nn.sigmoid(gg)
            act = (sg * uu).astype(jnp.bfloat16)
            out_ref[...] = (h1 + _dot(act, wd_ref[...])).astype(out_ref.dtype)

        with jax.named_scope("mlp_bwd"):
            dout_b = dout_ref[...]
            dout = dout_b.astype(jnp.float32)
            dact = _dot(dout_b, wd_ref[...], _NT)
            du = (dact * sg).astype(jnp.bfloat16)
            dg = (dact * uu * sg * (1.0 - sg)).astype(jnp.bfloat16)
            ad[...] += _dot(act, dout_b, _TN)
            hnT = hn.T.astype(jnp.bfloat16)
            ag[...] += _dot(hnT, dg)
            au[...] += _dot(hnT, du)
            dhn = _dot(dg, wg_ref[...]) + _dot(du, wu_ref[...])
            dh = dout + _ln_bwd(dhn, hn, r2)
            dh_s[slot] = dh
            dhb = dh.astype(jnp.bfloat16)
            ao[...] += _dot(oTb, dhb)
            doT_s[...] = _dot(wo_ref[...], dhb, _NT)

        @pl.when(i == NB - 1)
        def _write_mlp_grads():
            dwo_ref[...] = ao[...].astype(dwo_ref.dtype)
            dwg_ref[...] = ag[...].T.astype(dwg_ref.dtype)
            dwu_ref[...] = au[...].T.astype(dwu_ref.dtype)
            dwd_ref[...] = ad[...].astype(dwd_ref.dtype)
            for k in range(1, 5):
                out_copy(k).start()

        def att_bwd(b, carry):
            q0 = pl.multiple_of(b * QB, QB)
            s0 = pl.multiple_of(row0 + q0, QB)

            def wdo(g, hl):
                h = g * 8 + hl
                slab = (doT_s[pl.ds(h * DH, DH), pl.ds(q0, QB)] * rl_s[b, h:h + 1, :]).astype(jnp.bfloat16)
                return _head_w(slab, hl)

            def wq(g, hl):
                h = g * 8 + hl
                return _head_w(qT_s[pl.ds(h * DH, DH), pl.ds(q0, QB)], hl)

            for g in range(NG):
                vw = v_s[g, pl.ds(s0, NKEY), :]
                for hl in range(8):
                    h = g * 8 + hl
                    rows = pl.ds(h * DH, DH)
                    delta = jnp.sum(doT_s[rows, pl.ds(q0, QB)] * oT_s[rows, pl.ds(q0, QB)],
                                    axis=0, keepdims=True)
                    c = delta * rl_s[b, h:h + 1, :]
                    dpT = _dot(vw, wdo(g, hl))
                    p = p_s[b, g, :, hl * 128:(hl + 1) * 128].astype(jnp.float32)
                    ds_s[g, :, hl * 128:(hl + 1) * 128] = (p * (dpT - c)).astype(jnp.bfloat16)
            for g in range(NG):
                for hl in range(8):
                    h = g * 8 + hl
                    slab = (doT_s[pl.ds(h * DH, DH), pl.ds(q0, QB)] * rl_s[b, h:h + 1, :]).astype(jnp.bfloat16)
                    dvT_s[pl.ds(h * DH, DH), pl.ds(s0, NKEY)] += _dot(
                        slab, p_s[b, g, :, hl * 128:(hl + 1) * 128], _NT)
            for g in range(NG):
                for hl in range(8):
                    h = g * 8 + hl
                    kTw = kT_s[pl.ds(h * DH, DH), pl.ds(s0, NKEY)]
                    dqT_s[pl.ds(h * DH, DH), pl.ds(q0, QB)] = _dot(kTw, ds_s[g, :, hl * 128:(hl + 1) * 128])
            for g in range(NG):
                for hl in range(8):
                    h = g * 8 + hl
                    dkT_s[pl.ds(h * DH, DH), pl.ds(s0, NKEY)] += _dot(
                        qT_s[pl.ds(h * DH, DH), pl.ds(q0, QB)], ds_s[g, :, hl * 128:(hl + 1) * 128], _NT)
            return carry

        with jax.named_scope("att_bwd"):
            jax.lax.fori_loop(0, NSUB, att_bwd, 0)
            dq_s[slot] = dqT_s[...] * (DH ** -0.5)

    @pl.when(i >= 1)
    def _finalize():
        with jax.named_scope("finalize"):
            j = i - 1
            row0 = pl.multiple_of(j * TM, TM)
            slot = j % 2
            xn1 = xn_s[slot]
            r1 = r1_s[slot]
            dqkvT = jnp.concatenate([
                dq_s[slot].astype(jnp.bfloat16),
                (dkT_s[:, pl.ds(W + row0, TM)] * LN2).astype(jnp.bfloat16),
                dvT_s[:, pl.ds(W + row0, TM)].astype(jnp.bfloat16)], axis=0)
            aqkv[...] += _dot(dqkvT, xn1.astype(jnp.bfloat16))
            dxn1 = _dot(wqkv_ref[...], dqkvT).T
            dx_ref[...] = (dh_s[slot] + _ln_bwd(dxn1, xn1, r1)).astype(dx_ref.dtype)

    @pl.when(i == NB)
    def _write():
        dwqkv_ref[...] = aqkv[...].T.astype(dwqkv_ref.dtype)
        out_copy(0).start()
        for k in range(5):
            out_copy(k).wait()


@jax.jit
def pallas_sequential_preLN__sliding_block__glu_gated_glu__prompt_kernel(
    A_x: jax.Array,
    A_wqkv: jax.Array,
    A_wo: jax.Array,
    B_x: jax.Array,
    B_w_gate: jax.Array,
    B_w_up: jax.Array,
    B_w_down: jax.Array,
    grad_out: jax.Array,
):
    del B_x
    x2 = A_x.reshape(S, D)
    g2 = grad_out.reshape(S, D)
    bf = jnp.bfloat16
    f32 = jnp.float32

    cur = lambda i: (jnp.minimum(i, NB - 1), 0)
    lag = lambda i: (jnp.maximum(i - 1, 0), 0)
    const = lambda i: (0, 0)

    def wspec(shape):
        return pl.BlockSpec(shape, const, pipeline_mode=pl.Buffered(1))

    in_specs = [
        pl.BlockSpec((TM, D), cur),
        pl.BlockSpec((TM, D), cur),
    ] + [pl.BlockSpec(memory_space=pl.ANY)] * 5
    out_specs = [
        pl.BlockSpec((TM, D), cur),
        pl.BlockSpec((TM, D), lag),
    ] + [pl.BlockSpec(memory_space=pl.ANY)] * 5
    out_shape = [
        jax.ShapeDtypeStruct((S, D), bf),
        jax.ShapeDtypeStruct((S, D), bf),
        jax.ShapeDtypeStruct((D, 3 * D), bf),
        jax.ShapeDtypeStruct((D, D), bf),
        jax.ShapeDtypeStruct((F, D), bf),
        jax.ShapeDtypeStruct((F, D), bf),
        jax.ShapeDtypeStruct((F, D), bf),
    ]
    wshapes = [(D, 3 * D), (D, D), (F, D), (F, D), (F, D)]
    scratch = [pltpu.VMEM(sh, bf) for sh in wshapes] + [pltpu.VMEM(sh, bf) for sh in wshapes] + [
        pltpu.SemaphoreType.DMA((5,)),
        pltpu.SemaphoreType.DMA((5,)),
        pltpu.VMEM((D, TM), bf),
        pltpu.VMEM((NG, W + S, 128), bf),
        pltpu.VMEM((NG, W + S, 128), bf),
        pltpu.VMEM((D, W + S), bf),
        pltpu.VMEM((D, W + S), bf),
        pltpu.VMEM((D, TM), f32),
        pltpu.VMEM((NSUB, NG, NKEY, 8 * 128), bf),
        pltpu.VMEM((NG, NKEY, 8 * 128), bf),
        pltpu.VMEM((NSUB, H, 128), f32),
        pltpu.VMEM((D, TM), f32),
        pltpu.VMEM((D, TM), f32),
        pltpu.VMEM((NG, NKEY, 8 * 128), f32),
        pltpu.VMEM((H, 128), f32),
        pltpu.VMEM((D, W + S), f32),
        pltpu.VMEM((D, W + S), f32),
        pltpu.VMEM((2, D, TM), f32),
        pltpu.VMEM((2, TM, D), f32),
        pltpu.VMEM((2, TM, D), f32),
        pltpu.VMEM((2, TM, 1), f32),
        pltpu.VMEM((3 * D, D), f32),
        pltpu.VMEM((D, D), f32),
        pltpu.VMEM((D, F), f32),
        pltpu.VMEM((D, F), f32),
        pltpu.VMEM((F, D), f32),
    ]
    outs = pl.pallas_call(
        _kernel,
        grid=(NB + 1,),
        in_specs=in_specs,
        out_specs=out_specs,
        out_shape=out_shape,
        scratch_shapes=scratch,
        compiler_params=pltpu.CompilerParams(
            dimension_semantics=("arbitrary",),
            vmem_limit_bytes=100 * 1024 * 1024,
        ),
    )(x2, g2, A_wqkv, A_wo, B_w_gate.T, B_w_up.T, B_w_down)
    out, dx, dwqkv, dwo, dwg, dwu, dwd = outs
    return (out.reshape(1, S, D), dx.reshape(1, S, D), dwqkv, dwo, dwg.T, dwu.T, dwd)
```
